```python
import os as _os
_os.environ.setdefault("JAX_PLATFORMS", "cpu")
import jax
import jax.numpy as jnp

def _softmax(x, axis=-1):
    return jax.nn.softmax(x, axis=axis)
def _gelu(x):
    return jax.nn.gelu(x, approximate=True)
def _silu(x):
    return jax.nn.silu(x)
def _sigmoid(x):
    return jax.nn.sigmoid(x)
def _layernorm(x, axis=-1, eps=1e-5):
    m = jnp.mean(x, axis=axis, keepdims=True)
    v = jnp.var(x, axis=axis, keepdims=True)
    return (x - m) / jnp.sqrt(v + eps)
def _scatter_add(tgt, idx, src, axis=0):
    return tgt.at[idx].add(src)
def _segment_sum(src, seg, n):
    return jax.ops.segment_sum(src, seg, n)
class _Rng:
    def __init__(self, key):
        self._k = key
    def _next(self):
        self._k, sub = jax.random.split(self._k)
        return sub
    def normal(self, shape):
        return jax.random.normal(self._next(), shape, dtype=jnp.bfloat16)
    def randint(self, lo, hi, shape):
        return jax.random.randint(self._next(), shape, lo, hi, dtype=jnp.int32)
    def uniform(self, shape, lo=0.0, hi=1.0):
        return jax.random.uniform(self._next(), shape, jnp.bfloat16, lo, hi)
    def permutation(self, n):
        return jax.random.permutation(self._next(), n)


kernel_name = 'interleave_layers__sliding_block_cached__mixer_channel_mlp__decode'

def setup_inputs():
    _rng = _Rng(jax.random.key(int.from_bytes(__import__("os").urandom(4), "little")))
    _w = (lambda a: (lambda t: t.astype(jnp.bfloat16) if jnp.issubdtype(t.dtype, jnp.floating) else t)(jnp.asarray(a)))
    def _A_setup():
        B, Sq, D = 8, 1, 1024
        Hq, Hkv, Sk, Dh = 32, 4, 4096, 128
        assert Hq % Hkv == 0, (Hq, Hkv)
        return {
            "x": _w((lambda *s: _rng.normal(s) * 0.05)(B, Sq, D)),
            "k_cache": _w((lambda *s: _rng.normal(s) * 1.6)(B, Hkv, Sk, Dh)),
            "v_cache": _w((lambda *s: _rng.normal(s) * 0.8)(B, Hkv, Sk, Dh)),
            "wq": _w((lambda *s: _rng.normal(s) * 1.6)(D, Hq * Dh) * (D ** -0.5)),
            "wo": _w((lambda *s: _rng.normal(s) * 0.8)(Hq * Dh, D) * ((Hq * Dh) ** -0.5)),
        }
    _A_in = _A_setup()

    def _B_setup():
        B, S, D, F = 8, 1, 1024, 3584
        return {
            "x": _w((lambda *s: _rng.normal(s) * 0.05)(B, S, D)),
            "w1": _w((lambda *s: _rng.normal(s) * 0.4)(D, F) * (D ** -0.5)),
            "b1": _w((lambda *s: _rng.normal(s) * 0.4)(F)),
            "w2": _w((lambda *s: _rng.normal(s) * 0.4)(F, D) * (F ** -0.5)),
            "b2": _w((lambda *s: _rng.normal(s) * 0.1)(D)),
        }
    _B_in = _B_setup()

    return {
        "A_x": _A_in["x"],
        "A_k_cache": _A_in["k_cache"],
        "A_v_cache": _A_in["v_cache"],
        "A_wq": _A_in["wq"],
        "A_wo": _A_in["wo"],
        "B_x": _B_in["x"],
        "B_w1": _B_in["w1"],
        "B_b1": _B_in["b1"],
        "B_w2": _B_in["w2"],
        "B_b2": _B_in["b2"],
    }

def reference(A_x, A_k_cache, A_v_cache, A_wq, A_wo, B_x, B_w1, B_b1, B_w2, B_b2):
    def _A_ref(x, k_cache, v_cache, wq, wo):
        B, Sq, D = x.shape
        Hq, Dh = 32, 128
        Hkv, Sk = k_cache.shape[1], k_cache.shape[2]
        W = min(4096, max(256, Sk // 4))
        rep = Hq // Hkv
        q = (lambda x, *d: x.transpose(*d))((x @ wq).reshape(B, Sq, Hq, Dh), 0, 2, 1, 3)
        k = jnp.repeat(k_cache[:, :, Sk - W:, :], rep, axis=1)
        v = jnp.repeat(v_cache[:, :, Sk - W:, :], rep, axis=1)
        scores = jnp.einsum("bhqd,bhkd->bhqk", q, k) * (Dh ** -0.5)
        p = _softmax(scores, axis=-1)
        o = jnp.einsum("bhqk,bhkd->bhqd", p, v)
        return (lambda x, *d: x.transpose(*d))(o, 0, 2, 1, 3).reshape(B, Sq, Hq * Dh) @ wo

    def _B_ref(x, w1, b1, w2, b2):
        y = _layernorm(x, axis=-1)
        h = _gelu(jnp.einsum("bsd,df->bsf", y, w1) + b1)
        return jnp.einsum("bsf,fd->bsd", h, w2) + b2

    x = A_x
    x = x + _A_ref(_layernorm(x, axis=-1), A_k_cache, A_v_cache, A_wq, A_wo)
    x = x + _B_ref(_layernorm(x, axis=-1), B_w1, B_b1, B_w2, B_b2)
    x = x + _A_ref(_layernorm(x, axis=-1), A_k_cache, A_v_cache, A_wq, A_wo)
    x = x + _B_ref(_layernorm(x, axis=-1), B_w1, B_b1, B_w2, B_b2)
    return x
```

```python
import jax
import jax.numpy as jnp
from jax import lax
import jax.experimental.pallas as pl
import jax.experimental.pallas.tpu as pltpu

F32 = jnp.float32
BF16 = jnp.bfloat16
U32 = jnp.uint32

HQ, DH = 32, 128
EPS = 1e-5
W2_SPLIT = 768
W2_TAIL_ROWS = 512
LOOKAHEAD = 4


def _dot(a, b):
    return jnp.dot(a, b, preferred_element_type=F32)


def _ln_stats(x):
    m = jnp.mean(x, axis=-1, keepdims=True)
    d = x - m
    v = jnp.mean(d * d, axis=-1, keepdims=True)
    return m, lax.rsqrt(v + EPS)


def _layernorm(x):
    m, r = _ln_stats(x)
    return (x - m) * r


def _gelu(x):
    c = 0.7978845608028654
    return 0.5 * x * (1.0 + jnp.tanh(c * (x + 0.044715 * (x * x * x))))


def _w(ref, rows, cols):
    r0, nr = rows
    return pltpu.bitcast(ref[pl.ds(r0 // 2, nr // 2), cols], BF16)


def _kernel(x_h, k_h, v_h, wq_h, wo_h, w1_h, b1_h, w2_h, b2_h, out_h,
            x_v, b1_v, b2_v, wq_v, k_v, kt_v, v_v, wo_v, w1_v, w2_v,
            q_s, o_s, p_s, csq_s, cs1_s, b1_s, h_s, xr_s, qraw_s, out_v, sems):
    B, D = x_v.shape
    NU, W, _ = k_v.shape
    G = NU // B
    REP = HQ // G
    F = w1_v.shape[1]
    SK = k_h.shape[1]
    scale = DH ** -0.5
    CA = W2_SPLIT
    FT = F - W2_TAIL_ROWS

    w2u = w2_h.bitcast(U32)
    pairs = [
        (x_h, x_v),
        (wq_h.bitcast(U32), wq_v),
        (b1_h, b1_v),
        (b2_h, b2_v),
        (k_h.at[:, pl.ds(SK - W, W), :], k_v),
        (v_h.at[:, pl.ds(SK - W, W), :], v_v),
        (wo_h.bitcast(U32), wo_v),
        (w1_h.bitcast(U32), w1_v),
        (w2u.at[:, pl.ds(0, CA)], w2_v.at[:, pl.ds(0, CA)]),
        (w2u.at[pl.ds(0, FT // 2), pl.ds(CA, D - CA)],
         w2_v.at[pl.ds(0, FT // 2), pl.ds(CA, D - CA)]),
        (w2u.at[pl.ds(FT // 2, (F - FT) // 2), pl.ds(CA, D - CA)],
         w2_v.at[pl.ds(FT // 2, (F - FT) // 2), pl.ds(CA, D - CA)]),
    ]
    cps = [pltpu.make_async_copy(s, d, sems.at[i]) for i, (s, d) in enumerate(pairs)]
    for c in cps:
        c.start()
    (cp_x, cp_wq, cp_b1, cp_b2, cp_k, cp_v, cp_wo, cp_w1,
     cp_w2a, cp_w2b, cp_w2c) = cps

    ones = jnp.ones((B, D), F32)

    cp_x.wait()
    x0 = x_v[...].astype(F32)
    lhs_q = jnp.concatenate([_layernorm(x0), ones], axis=0).astype(BF16)
    cp_wq.wait()

    def q_body(n, c):
        cols = pl.ds(pl.multiple_of(n * 512, 512), 512)
        r = _dot(lhs_q, _w(wq_v, (0, D), cols))
        csq_s[:, cols] = r[B:]
        for j in range(4):
            q_s[pl.ds(n * 4 + j, B, stride=HQ), :] = r[:B, j * DH:(j + 1) * DH]
        return c
    lax.fori_loop(0, HQ // 4, q_body, 0)

    cp_b1.wait()
    cp_b2.wait()
    b1f = b1_v[...].astype(F32)
    for c in range(F // 128):
        b1_s[:, c * 128:(c + 1) * 128] = jnp.broadcast_to(b1f[c:c + 1, :], (B, 128))
    b2f = b2_v[...].astype(F32)
    b2row = jnp.concatenate(
        [jnp.broadcast_to(b2f[c:c + 1, :], (B, 128)) for c in range(D // 128)], axis=1)

    cp_k.wait()

    def qk_body(u, c):
        kt = k_v[u].T
        kt_v[u] = pltpu.bitcast(kt, U32)
        q = q_s[pl.ds(pl.multiple_of(u * REP, REP), REP), :].astype(BF16)
        s = _dot(q, kt) * scale
        p = jnp.exp(s - jnp.max(s, axis=-1, keepdims=True))
        p_s[u] = p / jnp.sum(p, axis=-1, keepdims=True)
        return c
    lax.fori_loop(0, NU, qk_body, 0)

    cp_v.wait()

    def pv_body(u, c):
        o = _dot(p_s[u].astype(BF16), v_v[u])
        o_s[pl.ds((u % G) * (REP * B) + u // G, REP, stride=B), :] = o
        return c
    lax.fori_loop(0, NU, pv_body, 0)

    o1 = jnp.concatenate([o_s[h * B:(h + 1) * B, :] for h in range(HQ)],
                         axis=1).astype(BF16)
    xr_s[...] = x0
    cp_wo.wait()

    def wo_body(n, c):
        cols = pl.ds(pl.multiple_of(n * 128, 128), 128)
        xr_s[:, cols] += _dot(o1, _w(wo_v, (0, HQ * DH), cols))
        return c
    lax.fori_loop(0, D // 128, wo_body, 0)

    x1 = xr_s[...]
    lhs_1 = jnp.concatenate([_layernorm(_layernorm(x1)), ones], axis=0).astype(BF16)
    xr_s[...] = x1 + b2row
    cp_w1.wait()

    def w1_body(n, c):
        cols = pl.ds(pl.multiple_of(n * 512, 512), 512)
        r = _dot(lhs_1, _w(w1_v, (0, D), cols))
        cs1_s[:, cols] = r[B:]
        h_s[:, cols] = _gelu(r[:B] + b1_s[:, cols])
        return c
    lax.fori_loop(0, F // 512, w1_body, 0)

    h1 = h_s[...].astype(BF16)
    cp_w2a.wait()

    def w2_body(n, c):
        cols = pl.ds(pl.multiple_of(n * 128, 128), 128)
        xr_s[:, cols] += _dot(h1, _w(w2_v, (0, F), cols))
        return c
    lax.fori_loop(0, CA // 128, w2_body, 0)

    x2a = xr_s[:, 0:CA].astype(BF16)

    def q2_body(n, c):
        cols = pl.ds(pl.multiple_of(n * 512, 512), 512)
        qraw_s[:, cols] = _dot(x2a, _w(wq_v, (0, CA), cols))
        return c
    lax.fori_loop(0, HQ // 4, q2_body, 0)

    cb = pl.ds(CA, D - CA)
    cp_w2b.wait()
    x2b = xr_s[:, cb] + _dot(h1[:, 0:FT], _w(w2_v, (0, FT), cb))
    cp_w2c.wait()

    x2b = (x2b + _dot(h1[:, FT:F], _w(w2_v, (FT, F - FT), cb))).astype(BF16)
    x2 = jnp.concatenate([x2a, x2b], axis=1).astype(F32)
    m2, r2 = _ln_stats(x2)

    def q_proj(g):
        cols = pl.ds(g * REP * DH, REP * DH)
        q = qraw_s[:, cols] + _dot(x2b, _w(wq_v, (CA, D - CA), cols))
        q = (q - m2 * csq_s[:, cols]) * r2
        for j in range(REP):
            q_s[pl.ds(g * REP + j, B, stride=HQ), :] = q[:, j * DH:(j + 1) * DH]

    def qk(g, b):
        u = b * G + g
        q = q_s[u * REP:(u + 1) * REP, :].astype(BF16)
        s = _dot(q, pltpu.bitcast(kt_v[u], BF16)) * scale
        p = jnp.exp(s - jnp.max(s, axis=-1, keepdims=True))
        return p.astype(BF16), 1.0 / jnp.sum(p, axis=-1, keepdims=True)

    def pv(g, b, p, inv):
        o = _dot(p, v_v[b * G + g]) * inv
        o_s[pl.ds(g * REP * B + b, REP, stride=B), :] = o

    def o_lhs(g):
        return jnp.concatenate(
            [o_s[(g * REP + j) * B:(g * REP + j + 1) * B, :] for j in range(REP)],
            axis=1).astype(BF16)

    def o_proj(g, lhs, c0, nc):
        return _dot(lhs, _w(wo_v, (g * REP * DH, REP * DH), pl.ds(c0, nc)))

    units = [(g, b) for g in range(G) for b in range(B)]
    for g in range(G):
        q_proj(g)
    pend = {}
    x3 = x2
    for i in range(NU + LOOKAHEAD):
        if i < NU:
            pend[i] = qk(*units[i])
        j = i - LOOKAHEAD
        if j >= 0:
            pv(*units[j], *pend.pop(j))
            if j % B == B // 2 and 1 <= j // B <= G - 2:
                g = j // B - 1
                x3 = x3 + o_proj(g, o_lhs(g), 0, D)
    x3 = x3 + o_proj(G - 2, o_lhs(G - 2), 0, D)
    ol = o_lhs(G - 1)
    HD = D // 2
    x3a = (x3[:, :HD] + o_proj(G - 1, ol, 0, HD)).astype(BF16)
    x3b = (x3[:, HD:] + o_proj(G - 1, ol, HD, HD)).astype(BF16)
    x3h = jnp.concatenate([x3a, x3b], axis=1)
    x3 = x3h.astype(F32)
    m3, r3 = _ln_stats(x3)
    m4, r4 = _ln_stats((x3 - m3) * r3)
    ln_a = r3 * r4
    ln_b = (m3 * r3 + m4) * r4

    FC = 512

    def mlp_up(c):
        cols = pl.ds(c * FC, FC)
        if c < 2:
            r = _dot(x3a, _w(w1_v, (0, HD), cols)) + _dot(x3b, _w(w1_v, (HD, HD), cols))
        else:
            r = _dot(x3h, _w(w1_v, (0, D), cols))
        return _gelu(r * ln_a - cs1_s[:, cols] * ln_b + b1_s[:, cols]).astype(BF16)

    nfc = F // FC
    hs = {}
    acc = x3 + b2row
    for c in range(nfc + 2):
        if c < nfc:
            hs[c] = mlp_up(c)
        if c >= 2:
            acc = acc + _dot(hs.pop(c - 2), _w(w2_v, ((c - 2) * FC, FC), pl.ds(0, D)))
    out_v[...] = acc.astype(out_v.dtype)
    cp_out = pltpu.make_async_copy(out_v, out_h, sems.at[len(cps)])
    cp_out.start()
    cp_out.wait()


@jax.jit
def pallas_interleave_layers__sliding_block_cached__mixer_channel_mlp__decode_kernel(
    A_x: jax.Array,
    A_k_cache: jax.Array,
    A_v_cache: jax.Array,
    A_wq: jax.Array,
    A_wo: jax.Array,
    B_x: jax.Array,
    B_w1: jax.Array,
    B_b1: jax.Array,
    B_w2: jax.Array,
    B_b2: jax.Array,
):
    del B_x
    B, Sq, D = A_x.shape
    _, Hkv, Sk, Dh = A_k_cache.shape
    F = B_w1.shape[1]
    W = min(4096, max(256, Sk // 4))
    NU = B * Hkv
    assert Sq == 1 and Dh == DH

    hbm = pl.BlockSpec(memory_space=pltpu.HBM)
    out = pl.pallas_call(
        _kernel,
        out_shape=jax.ShapeDtypeStruct((B, D), A_x.dtype),
        in_specs=[hbm] * 9,
        out_specs=hbm,
        scratch_shapes=[
            pltpu.VMEM((B, D), BF16),
            pltpu.VMEM((F // 128, 128), BF16),
            pltpu.VMEM((D // 128, 128), BF16),
            pltpu.VMEM((D // 2, HQ * DH), U32),
            pltpu.VMEM((NU, W, DH), BF16),
            pltpu.VMEM((NU, DH // 2, W), U32),
            pltpu.VMEM((NU, W, DH), BF16),
            pltpu.VMEM((HQ * DH // 2, D), U32),
            pltpu.VMEM((D // 2, F), U32),
            pltpu.VMEM((F // 2, D), U32),
            pltpu.VMEM((B * HQ, DH), F32),
            pltpu.VMEM((HQ * B, DH), F32),
            pltpu.VMEM((NU, HQ // Hkv, W), F32),
            pltpu.VMEM((B, HQ * DH), F32),
            pltpu.VMEM((B, F), F32),
            pltpu.VMEM((B, F), F32),
            pltpu.VMEM((B, F), F32),
            pltpu.VMEM((B, D), F32),
            pltpu.VMEM((B, HQ * DH), F32),
            pltpu.VMEM((B, D), A_x.dtype),
            pltpu.SemaphoreType.DMA((12,)),
        ],
        compiler_params=pltpu.CompilerParams(vmem_limit_bytes=100 * 1024 * 1024),
    )(
        A_x.reshape(B, D),
        A_k_cache.reshape(NU, Sk, Dh),
        A_v_cache.reshape(NU, Sk, Dh),
        A_wq,
        A_wo,
        B_w1,
        B_b1.reshape(F // 128, 128),
        B_w2,
        B_b2.reshape(D // 128, 128),
    )
    return out.reshape(B, Sq, D)
```

```python
import jax
import jax.numpy as jnp
from jax import lax
import jax.experimental.pallas as pl
import jax.experimental.pallas.tpu as pltpu

F32 = jnp.float32
BF16 = jnp.bfloat16
U32 = jnp.uint32

HQ, DH = 32, 128
EPS = 1e-5
W2_STAGES = (
    (0, 640, (0, 2560, 3584)),
    (640, 896, (0, 2048, 3584)),
    (896, 1024, (0, 2048, 3072, 3584)),
)
LOOKAHEAD = 5
FC = 512


def _dot(a, b):
    return jnp.dot(a, b, preferred_element_type=F32)


def _ln_stats(x):
    m = jnp.mean(x, axis=-1, keepdims=True)
    d = x - m
    v = jnp.mean(d * d, axis=-1, keepdims=True)
    return m, lax.rsqrt(v + EPS)


def _layernorm(x):
    m, r = _ln_stats(x)
    return (x - m) * r


def _gelu(x):
    c = 0.7978845608028654
    return 0.5 * x * (1.0 + jnp.tanh(c * (x + 0.044715 * (x * x * x))))


def _swap_sublanes(vs):
    sub = lax.broadcasted_iota(jnp.int32, vs[0].shape, 0)
    vs = list(vs)
    for d in (4, 2, 1):
        low = (sub & d) == 0
        for i in range(8):
            if not i & d:
                a, b = vs[i], vs[i + d]
                vs[i] = jnp.where(low, a, pltpu.roll(b, d, 0))
                vs[i + d] = jnp.where(low, pltpu.roll(a, 8 - d, 0), b)
    return vs


def _pieces(cuts):
    return list(zip(cuts[:-1], cuts[1:]))


def _w(packed, r0, r1, cols):
    return pltpu.bitcast(packed[r0 // 2:r1 // 2, cols], BF16)


def _w_repack(raw, packed, r0, r1, cols):
    w = raw[r0:r1, cols]
    packed[r0 // 2:r1 // 2, cols] = pltpu.bitcast(w, U32)
    return w


def _kernel(x_h, k_h, v_h, wq_h, wo_h, w1_h, b1_h, w2_h, b2_h, out_h,
            x_v, b1_v, b2_v, k_v, v_v, wq_r, wo_r, w1_r, w2_r,
            kt_p, wq_p, wo_p, w1_p, w2_p,
            q_s, o_s, p_s, csq_s, cs1_s, b1_s, h_s, xr_s, qraw_s, out_v, sems):
    B, D = x_v.shape
    NU, W, _ = k_v.shape
    G = NU // B
    REP = HQ // G
    GD = REP * DH
    F = w1_r.shape[1]
    SK = k_h.shape[1]
    scale = DH ** -0.5

    CL, _, last_cuts = W2_STAGES[-1]
    last_cols = pl.ds(CL, D - CL)
    cp_last = []
    for i, (r0, r1) in enumerate(_pieces(last_cuts)):
        blk = (pl.ds(r0, r1 - r0), last_cols)
        cp_last.append(pltpu.make_async_copy(w2_h.at[blk], w2_r.at[blk], sems.at[i]))

    def layer1(early_sems):
        pairs = [
            (wq_h, wq_r),
            (x_h, x_v),
            (b1_h, b1_v),
            (b2_h, b2_v),
            (k_h.at[:, pl.ds(SK - W, W), :], k_v),
            (v_h.at[:, pl.ds(SK - W, W), :], v_v),
            (wo_h, wo_r),
            (w1_h, w1_r),
        ]
        for c0, c1, cuts in W2_STAGES[:-1]:
            for r0, r1 in _pieces(cuts):
                blk = (pl.ds(r0, r1 - r0), pl.ds(c0, c1 - c0))
                pairs.append((w2_h.at[blk], w2_r.at[blk]))
        cps = [pltpu.make_async_copy(s, d, early_sems.at[i])
               for i, (s, d) in enumerate(pairs)]
        for cp in cps + cp_last:
            cp.start()
        cp_wq, cp_x, cp_b1, cp_b2, cp_k, cp_v, cp_wo, cp_w1 = cps[:8]
        cp_w2 = iter(cps[8:])

        ones = jnp.ones((B, D), F32)
        cp_x.wait()
        x0 = x_v[...].astype(F32)
        xr_s[...] = x0
        lhs_q = jnp.concatenate([_layernorm(x0), ones], axis=0).astype(BF16)
        cp_wq.wait()

        def q_body(n, carry):
            cols = pl.ds(pl.multiple_of(n * 4 * DH, 4 * DH), 4 * DH)
            r = _dot(lhs_q, _w_repack(wq_r, wq_p, 0, D, cols))
            csq_s[:, cols] = r[B:]
            for j in range(4):
                rows = pl.ds(pl.multiple_of((n * 4 + j) * B, B), B)
                q_s[rows, :] = r[:B, j * DH:(j + 1) * DH]
            return carry
        lax.fori_loop(0, HQ // 4, q_body, 0)

        cp_b1.wait()
        cp_b2.wait()
        b1f = b1_v[...].astype(F32)
        for c in range(F // 128):
            b1_s[:, c * 128:(c + 1) * 128] = jnp.broadcast_to(b1f[c:c + 1, :], (B, 128))
        b2f = b2_v[...].astype(F32)
        b2row = jnp.concatenate(
            [jnp.broadcast_to(b2f[c:c + 1, :], (B, 128)) for c in range(D // 128)], axis=1)

        cp_k.wait()

        def qk_body(u, carry):
            kt = k_v[u].T
            kt_p[u] = pltpu.bitcast(kt, U32)
            q = q_s[pl.ds((u % G) * (REP * B) + u // G, REP, stride=B), :]
            s = _dot(q.astype(BF16), kt) * scale
            p = jnp.exp(s - jnp.max(s, axis=-1, keepdims=True))
            p_s[u] = p / jnp.sum(p, axis=-1, keepdims=True)
            return carry
        lax.fori_loop(0, NU, qk_body, 0)

        cp_v.wait()

        def pv_body(u, carry):
            rows = pl.ds(pl.multiple_of(u * REP, REP), REP)
            o_s[rows, :] = _dot(p_s[u].astype(BF16), v_v[u])
            return carry
        lax.fori_loop(0, NU, pv_body, 0)

        o1 = jnp.concatenate(
            [o_s[pl.ds(h, B, stride=HQ), :] for h in range(HQ)], axis=1).astype(BF16)
        cp_wo.wait()

        def wo_body(n, carry):
            cols = pl.ds(pl.multiple_of(n * 128, 128), 128)
            xr_s[:, cols] += _dot(o1, _w_repack(wo_r, wo_p, 0, HQ * DH, cols))
            return carry
        lax.fori_loop(0, D // 128, wo_body, 0)

        x1 = xr_s[...]
        lhs_1 = jnp.concatenate([_layernorm(_layernorm(x1)), ones], axis=0).astype(BF16)
        xr_s[...] = x1 + b2row
        cp_w1.wait()

        def w1_body(n, carry):
            cols = pl.ds(pl.multiple_of(n * FC, FC), FC)
            r = _dot(lhs_1, _w_repack(w1_r, w1_p, 0, D, cols))
            cs1_s[:, cols] = r[B:]
            h_s[:, cols] = _gelu(r[:B] + b1_s[:, cols])
            return carry
        lax.fori_loop(0, F // FC, w1_body, 0)

        h1 = h_s[...].astype(BF16)
        x2s = []
        for si, (c0, c1, cuts) in enumerate(W2_STAGES[:-1]):
            for r0, r1 in _pieces(cuts):
                next(cp_w2).wait()

                def w2_body(n, carry):
                    cols = pl.ds(pl.multiple_of(c0 + n * 128, 128), 128)
                    xr_s[:, cols] += _dot(h1[:, r0:r1], _w_repack(w2_r, w2_p, r0, r1, cols))
                    return carry
                lax.fori_loop(0, (c1 - c0) // 128, w2_body, 0, unroll=(si, r0) != (0, 0))

            xs = xr_s[:, c0:c1].astype(BF16)
            x2s.append(xs)

            def q2_body(g, carry):
                cols = pl.ds(pl.multiple_of(g * GD, GD), GD)
                r = _dot(xs, _w(wq_p, c0, c1, cols))
                qraw_s[:, cols] = r if si == 0 else qraw_s[:, cols] + r
                return carry
            lax.fori_loop(0, G, q2_body, 0, unroll=si > 0)
        return h1, b2row, x2s

    n_early = 8 + sum(len(cuts) - 1 for _, _, cuts in W2_STAGES[:-1])
    h1, b2row, x2s = pl.run_scoped(layer1, pltpu.SemaphoreType.DMA((n_early,)))

    x2l = xr_s[:, last_cols]
    for cp_w2_last, (r0, r1) in zip(cp_last, _pieces(last_cuts)):
        cp_w2_last.wait()
        x2l = x2l + _dot(h1[:, r0:r1], w2_r[r0:r1, last_cols])
    x2l = x2l.astype(BF16)

    x2 = jnp.concatenate([t.astype(F32) for t in x2s + [x2l]], axis=1)
    m2, r2 = _ln_stats(x2)
    s2 = r2 * scale
    q2 = []
    for g in range(G):
        cols = pl.ds(g * GD, GD)
        q = qraw_s[:, cols] + _dot(x2l, _w(wq_p, CL, D, cols)) - m2 * csq_s[:, cols]
        q2.append(_swap_sublanes([q[:, j * DH:(j + 1) * DH] for j in range(REP)]))

    def qk(g, b):
        kt = pltpu.bitcast(kt_p[b * G + g], BF16)
        s = _dot(q2[g][b].astype(BF16), kt) * s2[b:b + 1]
        p = jnp.exp(s - jnp.max(s, axis=-1, keepdims=True))
        return p.astype(BF16), 1.0 / jnp.sum(p, axis=-1, keepdims=True)

    o2 = {}

    def o_lhs(g):
        heads = _swap_sublanes([o2.pop((g, b)) for b in range(B)])
        return jnp.concatenate(heads, axis=1).astype(BF16)

    def o_proj(g, lhs, c0, c1):
        return _dot(lhs, _w(wo_p, g * GD, (g + 1) * GD, pl.ds(c0, c1 - c0)))

    units = [(g, b) for g in range(G) for b in range(B)]
    probs = {}
    x3 = x2
    for i in range(NU + LOOKAHEAD):
        if B <= i < B + F // FC:
            _w_repack(w2_r, w2_p, (i - B) * FC, (i - B + 1) * FC, last_cols)
        if i < NU:
            probs[i] = qk(*units[i])
        j = i - LOOKAHEAD
        if j >= 0:
            g, b = units[j]
            p, inv = probs.pop(j)
            o2[g, b] = _dot(p, v_v[b * G + g]) * inv
            if b == B // 2 and 1 <= g <= G - 2:
                x3 = x3 + o_proj(g - 1, o_lhs(g - 1), 0, D)
    x3 = x3 + o_proj(G - 2, o_lhs(G - 2), 0, D)
    ol = o_lhs(G - 1)
    HD = D // 2
    x3a = (x3[:, :HD] + o_proj(G - 1, ol, 0, HD)).astype(BF16)
    x3b = (x3[:, HD:] + o_proj(G - 1, ol, HD, D)).astype(BF16)
    x3h = jnp.concatenate([x3a, x3b], axis=1)
    x3 = x3h.astype(F32)

    m3, r3 = _ln_stats(x3)
    m4, r4 = _ln_stats((x3 - m3) * r3)
    ln_a = r3 * r4
    ln_b = (m3 * r3 + m4) * r4

    lag = 2
    r_head = _dot(x3a, _w(w1_p, 0, HD, pl.ds(0, lag * FC)))
    hs = {}
    acc = x3 + b2row
    for c in range(F // FC + lag):
        if c < F // FC:
            cols = pl.ds(c * FC, FC)
            if c < lag:
                r = r_head[:, c * FC:(c + 1) * FC] + _dot(x3b, _w(w1_p, HD, D, cols))
            else:
                r = _dot(x3h, _w(w1_p, 0, D, cols))
            hs[c] = _gelu(r * ln_a - cs1_s[:, cols] * ln_b + b1_s[:, cols]).astype(BF16)
        if c >= lag:
            r0 = (c - lag) * FC
            acc = acc + _dot(hs.pop(c - lag), _w(w2_p, r0, r0 + FC, pl.ds(0, D)))

    out_v[...] = acc.astype(out_v.dtype)
    cp_out = pltpu.make_async_copy(out_v, out_h, sems.at[0])
    cp_out.start()
    cp_out.wait()


@jax.jit
def pallas_interleave_layers__sliding_block_cached__mixer_channel_mlp__decode_kernel(
    A_x: jax.Array,
    A_k_cache: jax.Array,
    A_v_cache: jax.Array,
    A_wq: jax.Array,
    A_wo: jax.Array,
    B_x: jax.Array,
    B_w1: jax.Array,
    B_b1: jax.Array,
    B_w2: jax.Array,
    B_b2: jax.Array,
):
    del B_x
    B, Sq, D = A_x.shape
    _, Hkv, Sk, Dh = A_k_cache.shape
    F = B_w1.shape[1]
    W = min(4096, max(256, Sk // 4))
    NU = B * Hkv
    assert Sq == 1 and Dh == DH and B == 8 and HQ // Hkv == 8

    hbm = pl.BlockSpec(memory_space=pltpu.HBM)
    out = pl.pallas_call(
        _kernel,
        out_shape=jax.ShapeDtypeStruct((B, D), A_x.dtype),
        in_specs=[hbm] * 9,
        out_specs=hbm,
        scratch_shapes=[
            pltpu.VMEM((B, D), BF16),
            pltpu.VMEM((F // 128, 128), BF16),
            pltpu.VMEM((D // 128, 128), BF16),
            pltpu.VMEM((NU, W, DH), BF16),
            pltpu.VMEM((NU, W, DH), BF16),
            pltpu.VMEM((D, HQ * DH), BF16),
            pltpu.VMEM((HQ * DH, D), BF16),
            pltpu.VMEM((D, F), BF16),
            pltpu.VMEM((F, D), BF16),
            pltpu.VMEM((NU, DH // 2, W), U32),
            pltpu.VMEM((D // 2, HQ * DH), U32),
            pltpu.VMEM((HQ * DH // 2, D), U32),
            pltpu.VMEM((D // 2, F), U32),
            pltpu.VMEM((F // 2, D), U32),
            pltpu.VMEM((HQ * B, DH), F32),
            pltpu.VMEM((B * HQ, DH), F32),
            pltpu.VMEM((NU, HQ // Hkv, W), F32),
            pltpu.VMEM((B, HQ * DH), F32),
            pltpu.VMEM((B, F), F32),
            pltpu.VMEM((B, F), F32),
            pltpu.VMEM((B, F), F32),
            pltpu.VMEM((B, D), F32),
            pltpu.VMEM((B, HQ * DH), F32),
            pltpu.VMEM((B, D), A_x.dtype),
            pltpu.SemaphoreType.DMA((len(W2_STAGES[-1][2]) - 1,)),
        ],
        compiler_params=pltpu.CompilerParams(vmem_limit_bytes=100 * 1024 * 1024),
    )(
        A_x.reshape(B, D),
        A_k_cache.reshape(NU, Sk, Dh),
        A_v_cache.reshape(NU, Sk, Dh),
        A_wq,
        A_wo,
        B_w1,
        B_b1.reshape(F // 128, 128),
        B_w2,
        B_b2.reshape(D // 128, 128),
    )
    return out.reshape(B, Sq, D)
```
